```python
import os as _os
_os.environ.setdefault("JAX_PLATFORMS", "cpu")
import jax
import jax.numpy as jnp

def _softmax(x, axis=-1):
    return jax.nn.softmax(x, axis=axis)
def _gelu(x):
    return jax.nn.gelu(x, approximate=True)
def _silu(x):
    return jax.nn.silu(x)
def _sigmoid(x):
    return jax.nn.sigmoid(x)
def _layernorm(x, axis=-1, eps=1e-5):
    m = jnp.mean(x, axis=axis, keepdims=True)
    v = jnp.var(x, axis=axis, keepdims=True)
    return (x - m) / jnp.sqrt(v + eps)
def _scatter_add(tgt, idx, src, axis=0):
    return tgt.at[idx].add(src)
def _segment_sum(src, seg, n):
    return jax.ops.segment_sum(src, seg, n)
class _Rng:
    def __init__(self, key):
        self._k = key
    def _next(self):
        self._k, sub = jax.random.split(self._k)
        return sub
    def normal(self, shape):
        return jax.random.normal(self._next(), shape, dtype=jnp.bfloat16)
    def randint(self, lo, hi, shape):
        return jax.random.randint(self._next(), shape, lo, hi, dtype=jnp.int32)
    def uniform(self, shape, lo=0.0, hi=1.0):
        return jax.random.uniform(self._next(), shape, jnp.bfloat16, lo, hi)
    def permutation(self, n):
        return jax.random.permutation(self._next(), n)


kernel_name = 'gated_mix__compressed_kv_cla__linear_attn_block__prompt'

def setup_inputs():
    _rng = _Rng(jax.random.key(int.from_bytes(__import__("os").urandom(4), "little")))
    _w = (lambda a: (lambda t: t.astype(jnp.bfloat16) if jnp.issubdtype(t.dtype, jnp.floating) else t)(jnp.asarray(a)))
    def _A_setup():
        B, H, Sq, Sk, D, M = 1, 16, 2048, 2048, 256, 448
        Dc = 4 * D
        return {
            "x": _w((lambda *s: _rng.normal(s) * 0.05)(B, Sq, M)),
            "c_kv": _w((lambda *s: _rng.normal(s) * 0.8)(B, Sk, Dc)),
            "w_q": _w((lambda *s: _rng.normal(s) * 3.2)(M, H, D) * (M ** -0.5)),
            "w_uk": _w((lambda *s: _rng.normal(s) * 3.2)(Dc, H, D) * (Dc ** -0.5)),
            "w_uv": _w((lambda *s: _rng.normal(s) * 0.8)(Dc, H, D) * (Dc ** -0.5)),
            "w_o": _w((lambda *s: _rng.normal(s) * 0.8)(H, D, M) * ((H * D) ** -0.5)),
        }
    _A_in = _A_setup()

    def _B_setup():
        B, S, D = 1, 2048, 448
        return {
            "x": _w((lambda *s: _rng.normal(s) * 0.05)(B, S, D)),
            "wqkv": _w((lambda *s: _rng.normal(s) * 1.6)(D, 3 * D)),
            "wo": _w((lambda *s: _rng.normal(s) * 0.4)(D, D)),
        }
    _B_in = _B_setup()

    return {
        "A_x": _A_in["x"],
        "A_c_kv": _A_in["c_kv"],
        "A_w_q": _A_in["w_q"],
        "A_w_uk": _A_in["w_uk"],
        "A_w_uv": _A_in["w_uv"],
        "A_w_o": _A_in["w_o"],
        "B_x": _B_in["x"],
        "B_wqkv": _B_in["wqkv"],
        "B_wo": _B_in["wo"],
        "gate_w": _w((lambda *s: _rng.normal(s) * 0.05)(448) * 16.0),
    }

def reference(A_x, A_c_kv, A_w_q, A_w_uk, A_w_uv, A_w_o, B_x, B_wqkv, B_wo, gate_w):
    def _A_ref(x, c_kv, w_q, w_uk, w_uv, w_o):
        B, Sq, M = x.shape[0], x.shape[1], x.shape[2]
        Sk = c_kv.shape[1]
        H, D = w_q.shape[1], w_q.shape[2]
        q = jnp.einsum("bqm,mhd->bhqd", x, w_q)
        k = jnp.einsum("bkc,chd->bhkd", c_kv, w_uk)
        v = jnp.einsum("bkc,chd->bhkd", c_kv, w_uv)
        scores = jnp.einsum("bhqd,bhkd->bhqk", q, k) * (D ** -0.5)
        off = Sk - Sq
        qi = jnp.arange(Sq)[:, None]
        kj = jnp.arange(Sk)[None, :]
        cmask = kj <= (qi + off)
        scores = jnp.where(cmask[None, None], scores, -1e9)
        p = _softmax(scores, axis=-1)
        ctx = jnp.einsum("bhqk,bhkd->bhqd", p, v)
        return jnp.einsum("bhqd,hdm->bqm", ctx, w_o)

    def _B_ref(x, wqkv, wo):
        B, S, D = x.shape
        H = 16; Dh = D // H
        qkv = (lambda x, *d: x.transpose(*d))((x @ wqkv).reshape(B, S, 3, H, Dh), 2, 0, 3, 1, 4)
        q, k, v = qkv[0], qkv[1], qkv[2]
        phi = lambda t: jnp.where(t > 0, t + 1, jnp.exp(t)) + 1e-6
        pq, pk = phi(q), phi(k)
        kv = jnp.einsum("bhsd,bhse->bhde", pk, v)
        z = jnp.einsum("bhsd->bhd", pk)
        num = jnp.einsum("bhqd,bhde->bhqe", pq, kv)
        den = jnp.einsum("bhqd,bhd->bhq", pq, z)[..., None] + 1e-6
        o = num / den
        return (lambda x, *d: x.transpose(*d))(o, 0, 2, 1, 3).reshape(B, S, D) @ wo

    x = A_x
    g = _sigmoid((x * gate_w).sum(-1, keepdims=True))
    a = _A_ref(x, A_c_kv, A_w_q, A_w_uk, A_w_uv, A_w_o)
    b = _B_ref(x, B_wqkv, B_wo)
    return g * a + (1 - g) * b
```

```python
import os
import jax
import jax.numpy as jnp
from jax import lax
import jax.experimental.pallas as pl
import jax.experimental.pallas.tpu as pltpu

F32 = jnp.float32
BF16 = jnp.bfloat16
U32 = jnp.uint32

S = 2048
M = 448
H = 16
D = 256
DC = 1024
HB = 16
DH = M // HB
TQ = int(os.environ.get("TQ", "128"))
NQ = S // TQ
CB = int(os.environ.get("CB", "512"))
LA = int(os.environ.get("LA", "12"))
NSTEPS = int(os.environ.get("NSTEPS", "16"))

NT = (((1,), (1,)), ((), ()))
TN = (((0,), (0,)), ((), ()))

_DT = [(0, 128), (128, 256), (256, 384), (384, 448)]
_ER = []
for (_d0, _d1) in _DT:
    _h0, _h1 = _d0 // DH, (_d1 - 1) // DH
    _ER.append(((_h0 * DH) // 16 * 16, -(-((_h1 + 1) * DH) // 16) * 16))


def _dot(a, b):
    return jnp.dot(a, b, preferred_element_type=F32)


def _kernel(xT_ref, c_hbm, wq_hbm, wk_hbm, wv_hbm, woT_ref, wqkv_ref, wob_ref, gw_ref,
            out_ref, c_s, wq_b, wk_b, wv_b, sems, qT_s, k_s, vT_s, ctxT_s, acc_s,
            wT_s, kvz0, kvz1, kvz2, kvz3, pqT_s, kz0, kz1, kz2, kz3, wobT_s, bg_s, g_s):
    h = pl.program_id(0)
    j = h // 2
    slot = j % 2
    kvz = (kvz0, kvz1, kvz2, kvz3)
    kz = (kz0, kz1, kz2, kz3)

    def copies(jj, sl):
        return [
            pltpu.make_async_copy(wk_hbm.bitcast(U32).at[:, jj, :], wk_b.at[sl], sems.at[sl * 3 + 0]),
            pltpu.make_async_copy(wv_hbm.bitcast(U32).at[:, jj, :], wv_b.at[sl], sems.at[sl * 3 + 1]),
            pltpu.make_async_copy(wq_hbm.bitcast(U32).at[:, jj, :], wq_b.at[sl], sems.at[sl * 3 + 2]),
        ]

    c_copy = pltpu.make_async_copy(c_hbm.at[0], c_s, sems.at[6])

    @pl.when(h == 0)
    def _():
        c_copy.start()
        for cp in copies(0, 0):
            cp.start()

        def phi(t):
            return jnp.where(t > 0, t + 1.0, jnp.exp(t)) + 1e-6

        wT_s[0:3 * M, :] = wqkv_ref[...].astype(F32).T.astype(BF16)
        wT_s[3 * M:3 * M + 16, :] = jnp.broadcast_to(gw_ref[...], (16, M))
        wobT_s[...] = wob_ref[...].astype(F32).T.astype(BF16)
        for t in range(4):
            kvz[t][...] = jnp.zeros_like(kvz[t])

        def phase1(t, carry):
            off = pl.multiple_of(t * CB, CB)
            xT = xT_ref[:, pl.ds(off, CB)]
            qkvT = _dot(wT_s[...], xT)
            qbT = qkvT[0:M].astype(BF16).astype(F32)
            kbT = qkvT[M:2 * M].astype(BF16).astype(F32)
            vbT = qkvT[2 * M:3 * M].astype(BF16)
            g_s[:, pl.ds(off, CB)] = jax.nn.sigmoid(qkvT[3 * M:3 * M + 8])
            pqT_s[:, pl.ds(off, CB)] = phi(qbT).astype(BF16)
            pkT = phi(kbT).astype(BF16)
            ones = jnp.ones((16, CB), BF16)
            for tt in range(4):
                (d0, d1), (e0, e1) = _DT[tt], _ER[tt]
                vaug = jnp.concatenate([vbT[e0:e1], ones], axis=0)
                kvz[tt][...] += lax.dot_general(vaug, pkT[d0:d1], NT, preferred_element_type=F32)
            return carry

        lax.fori_loop(0, S // CB, phase1, 0)

        for tt in range(4):
            (d0, d1), (e0, e1) = _DT[tt], _ER[tt]
            ne = e1 - e0
            r = (lax.broadcasted_iota(jnp.int32, (ne, d1 - d0), 0) + e0) // DH
            cc = (lax.broadcasted_iota(jnp.int32, (ne, d1 - d0), 1) + d0) // DH
            same = r == cc
            kz[tt][0:ne, :] = jnp.where(same, kvz[tt][0:ne, :], 0.0).astype(BF16)
            kz[tt][ne:2 * ne, :] = jnp.where(same, kvz[tt][ne:ne + 1, :], 0.0).astype(BF16)

        def phase2(t, carry):
            off = pl.multiple_of(t * CB, CB)
            nd = []
            for tt in range(4):
                d0, d1 = _DT[tt]
                nd.append(_dot(kz[tt][...], pqT_s[d0:d1, pl.ds(off, CB)]))
            pieces = []
            cuts = sorted(set([e for er in _ER for e in er]))
            for a, b in zip(cuts[:-1], cuts[1:]):
                num = None
                den = None
                for tt in range(4):
                    e0, e1 = _ER[tt]
                    if e0 <= a and b <= e1:
                        ne = e1 - e0
                        n_ = nd[tt][a - e0:b - e0]
                        d_ = nd[tt][ne + a - e0:ne + b - e0]
                        num = n_ if num is None else num + n_
                        den = d_ if den is None else den + d_
                pieces.append((num / (den + 1e-6)).astype(BF16))
            oT = jnp.concatenate(pieces, axis=0)
            bT = _dot(wobT_s[...], oT)
            g = g_s[0:1, pl.ds(off, CB)]
            bg_s[:, pl.ds(off, CB)] = (1.0 - g) * bT
            return carry

        lax.fori_loop(0, S // CB, phase2, 0)
        acc_s[...] = jnp.zeros_like(acc_s)
        c_copy.wait()

    @pl.when(h % 2 == 0)
    def _():
        for cp in copies(j, slot):
            cp.wait()

        @pl.when(j + 1 < NSTEPS // 2)
        def _():
            for cp in copies(j + 1, 1 - slot):
                cp.start()

    shift = ((1 - h % 2) * 16).astype(U32)

    def unpack(buf):
        u = buf[slot]
        return lax.bitcast_convert_type((u << shift) & jnp.uint32(0xFFFF0000), F32)

    c = c_s[...]
    k_s[...] = _dot(c, unpack(wk_b).astype(BF16)).astype(BF16)
    vT_s[...] = _dot(c, unpack(wv_b).astype(BF16)).T.astype(BF16)
    wqT = unpack(wq_b).T.astype(BF16)
    qT_s[...] = (_dot(wqT, xT_ref[...]) * (D ** -0.5)).astype(BF16)

    krow = lax.broadcasted_iota(jnp.int32, (TQ, TQ), 0)
    qcol = lax.broadcasted_iota(jnp.int32, (TQ, TQ), 1)
    causal = krow <= qcol

    def scores(i):
        lo = i * TQ
        qT = qT_s[:, lo:lo + TQ]
        s_d = _dot(k_s[lo:lo + TQ, :], qT)
        s_d = jnp.where(causal, s_d, -1e9)
        m = jnp.max(s_d, axis=0, keepdims=True)
        s_o = None
        if i > 0:
            s_o = _dot(k_s[0:lo, :], qT)
            m = jnp.maximum(m, jnp.max(s_o, axis=0, keepdims=True))
        return s_d, s_o, m

    def finish(i, s_d, s_o, m):
        lo = i * TQ
        p_d = jnp.exp(s_d - m)
        l = jnp.sum(p_d, axis=0, keepdims=True)
        ctxT = _dot(vT_s[:, lo:lo + TQ], p_d.astype(BF16))
        if i > 0:
            p_o = jnp.exp(s_o - m)
            l = l + jnp.sum(p_o, axis=0, keepdims=True)
            ctxT = ctxT + _dot(vT_s[:, 0:lo], p_o.astype(BF16))
        ctxT_s[:, lo:lo + TQ] = (ctxT / l).astype(BF16)

    pend = [scores(i) for i in range(LA)]
    for i in range(NQ):
        if i + LA < NQ:
            pend.append(scores(i + LA))
        finish(i, *pend.pop(0))

    acc_s[...] += _dot(woT_ref[...], ctxT_s[...])

    @pl.when(h == NSTEPS - 1)
    def _():
        out_ref[...] = (g_s[0:1, :] * acc_s[...] + bg_s[...]).astype(out_ref.dtype)


def _build(interpret=False):
    ne = [e1 - e0 for (e0, e1) in _ER]
    nd = [d1 - d0 for (d0, d1) in _DT]
    return pl.pallas_call(
        _kernel,
        grid=(NSTEPS,),
        in_specs=[
            pl.BlockSpec((None, M, S), lambda h: (0, 0, 0)),
            pl.BlockSpec(memory_space=pl.ANY),
            pl.BlockSpec(memory_space=pl.ANY),
            pl.BlockSpec(memory_space=pl.ANY),
            pl.BlockSpec(memory_space=pl.ANY),
            pl.BlockSpec((None, M, D), lambda h: (h, 0, 0)),
            pl.BlockSpec((M, 3 * M), lambda h: (0, 0)),
            pl.BlockSpec((M, M), lambda h: (0, 0)),
            pl.BlockSpec((1, M), lambda h: (0, 0)),
        ],
        out_specs=pl.BlockSpec((None, M, S), lambda h: (0, 0, 0)),
        out_shape=jax.ShapeDtypeStruct((1, M, S), BF16),
        scratch_shapes=[
            pltpu.VMEM((S, DC), BF16),
            pltpu.VMEM((2, M, D), U32),
            pltpu.VMEM((2, DC, D), U32),
            pltpu.VMEM((2, DC, D), U32),
            pltpu.SemaphoreType.DMA((7,)),
            pltpu.VMEM((D, S), BF16),
            pltpu.VMEM((S, D), BF16),
            pltpu.VMEM((D, S), BF16),
            pltpu.VMEM((D, S), BF16),
            pltpu.VMEM((M, S), F32),
            pltpu.VMEM((3 * M + 16, M), BF16),
        ] + [pltpu.VMEM((ne[t] + 16, nd[t]), F32) for t in range(4)] + [
            pltpu.VMEM((M, S), BF16),
        ] + [pltpu.VMEM((2 * ne[t], nd[t]), BF16) for t in range(4)] + [
            pltpu.VMEM((M, M), BF16),
            pltpu.VMEM((M, S), F32),
            pltpu.VMEM((8, S), F32),
        ],
        compiler_params=pltpu.CompilerParams(
            dimension_semantics=("arbitrary",),
            vmem_limit_bytes=100 * 1024 * 1024,
        ),
        interpret=interpret,
    )


@jax.jit
def pallas_gated_mix__compressed_kv_cla__linear_attn_block__prompt_kernel(
    A_x, A_c_kv, A_w_q, A_w_uk, A_w_uv, A_w_o, B_x, B_wqkv, B_wo, gate_w,
):
    gw = gate_w.reshape(1, M)
    xT = jnp.swapaxes(A_x, 1, 2)
    woT = jnp.swapaxes(A_w_o, 1, 2)
    outT = _build()(xT, A_c_kv, A_w_q, A_w_uk, A_w_uv, woT, B_wqkv, B_wo, gw)
    return jnp.swapaxes(outT, 1, 2)
```

```python
import jax
import jax.numpy as jnp
from jax import lax
import jax.experimental.pallas as pl
import jax.experimental.pallas.tpu as pltpu

F32 = jnp.float32
BF16 = jnp.bfloat16
U32 = jnp.uint32

S = 2048
M = 448
H = 16
D = 256
DC = 1024
HB = 16
DH = M // HB
TQ = 128
NQ = S // TQ
CB = 512
NCB = S // CB

NT = (((1,), (1,)), ((), ()))
TN = (((0,), (0,)), ((), ()))

_DT = [(0, 128), (128, 256), (256, 384), (384, 448)]
_ER = []
for (_d0, _d1) in _DT:
    _h0, _h1 = _d0 // DH, (_d1 - 1) // DH
    _ER.append(((_h0 * DH) // 16 * 16, -(-((_h1 + 1) * DH) // 16) * 16))

SEM_W = 0
SEM_C = 8
SEM_WQKV = 9
SEM_WOB = 10
SEM_X = 11
SEM_O = SEM_X + NCB
NSEM = SEM_O + NCB

GROW = 2 * M
VROW = 2 * M + 16


def _dot(a, b):
    return jnp.dot(a, b, preferred_element_type=F32)


def _kernel(xT_hbm, c_hbm, wq_hbm, wk_hbm, wv_hbm, woT_hbm, wqkv_hbm, wob_hbm, gw_ref,
            out_hbm,
            xT_s, c_s, wqkv_s, wob_s, woT_b, wq_b, wk_b, wv_b, sems,
            qT_s, k_s, vT_s, ctxT_s, acc_s,
            wT_s, xp_s, pqT_s, z16_s, zm_s, e2_s, mk0, mk1, mk2, mk3, wk2_s, g_s, o_s):
    mk = (mk0, mk1, mk2, mk3)

    def w_copies(jj, sl):
        return [
            pltpu.make_async_copy(wk_hbm.bitcast(U32).at[:, jj, :], wk_b.at[sl], sems.at[SEM_W + sl * 4 + 0]),
            pltpu.make_async_copy(wv_hbm.bitcast(U32).at[:, jj, :], wv_b.at[sl], sems.at[SEM_W + sl * 4 + 1]),
            pltpu.make_async_copy(wq_hbm.bitcast(U32).at[:, jj, :], wq_b.at[sl], sems.at[SEM_W + sl * 4 + 2]),
            pltpu.make_async_copy(woT_hbm.at[pl.ds(2 * jj, 2)], woT_b.at[sl], sems.at[SEM_W + sl * 4 + 3]),
        ]

    def x_copy(t):
        off = pl.multiple_of(t * CB, CB)
        return pltpu.make_async_copy(xT_hbm.at[0, :, pl.ds(off, CB)], xT_s.at[:, pl.ds(off, CB)],
                                     sems.at[SEM_X + t])

    def o_copy(t):
        off = pl.multiple_of(t * CB, CB)
        return pltpu.make_async_copy(o_s.at[:, pl.ds(off, CB)], out_hbm.at[0, :, pl.ds(off, CB)],
                                     sems.at[SEM_O + t])

    c_copy = pltpu.make_async_copy(c_hbm.at[0], c_s, sems.at[SEM_C])
    wqkv_copy = pltpu.make_async_copy(wqkv_hbm, wqkv_s, sems.at[SEM_WQKV])
    wob_copy = pltpu.make_async_copy(wob_hbm, wob_s, sems.at[SEM_WOB])
    wqkv_copy.start()
    x_copy(0).start()
    wob_copy.start()

    def phi(t):
        return jnp.where(t > 0, t + 1.0, jnp.exp(t)) + 1e-6

    xp_s[...] = jnp.zeros_like(xp_s)
    acc_s[...] = jnp.zeros_like(acc_s)
    for tt in range(4):
        (d0, d1), (e0, e1) = _DT[tt], _ER[tt]
        r = (lax.broadcasted_iota(jnp.int32, (e1 - e0, d1 - d0), 0) + e0) // DH
        cc = (lax.broadcasted_iota(jnp.int32, (e1 - e0, d1 - d0), 1) + d0) // DH
        mk[tt][...] = jnp.where(r == cc, 1.0, 0.0)
    hrow = lax.broadcasted_iota(jnp.int32, (16, M), 0)
    hcol = lax.broadcasted_iota(jnp.int32, (16, M), 1) // DH
    zm_s[...] = jnp.where(hrow == hcol, 1.0, 0.0)
    erow = lax.broadcasted_iota(jnp.int32, (M, 32), 0) // DH
    ecol = lax.broadcasted_iota(jnp.int32, (M, 32), 1) % 16
    e2_s[...] = jnp.where(erow == ecol, 1.0, 0.0).astype(BF16)
    wT_s[GROW:GROW + 16, :] = jnp.broadcast_to(gw_ref[...].reshape(1, M), (16, M))

    wqkv_copy.wait()
    for t in range(1, NCB):
        x_copy(t).start()
    c_copy.start()
    for cp in w_copies(0, 0):
        cp.start()
    wT = wqkv_s[...].astype(F32).T.astype(BF16)
    wT_s[0:2 * M, :] = wT[0:2 * M]
    wT_s[VROW:VROW + M, :] = wT[2 * M:3 * M]

    def phase1(t, carry):
        off = pl.multiple_of(t * CB, CB)
        x_copy(t).wait()
        xT = xT_s[:, pl.ds(off, CB)]
        qkT = _dot(wT_s[0:VROW, :], xT)
        qbT = qkT[0:M].astype(BF16).astype(F32)
        kbT = qkT[M:2 * M].astype(BF16).astype(F32)
        g_s[:, pl.ds(off, CB)] = jax.nn.sigmoid(qkT[GROW:GROW + 8])
        pqT_s[:, pl.ds(off, CB)] = phi(qbT).astype(BF16)
        pkT = phi(kbT).astype(BF16)
        xaug = jnp.concatenate([xT, jnp.ones((16, CB), BF16)], axis=0)
        xp_s[...] += lax.dot_general(xaug, pkT, NT, preferred_element_type=F32)
        return carry

    lax.fori_loop(0, NCB, phase1, 0)

    wob_copy.wait()
    for tt in range(4):
        (d0, d1), (e0, e1) = _DT[tt], _ER[tt]
        kvT = _dot(wT_s[VROW + e0:VROW + e1, :], xp_s[0:M, d0:d1].astype(BF16))
        kvT = jnp.where(mk[tt][...] > 0.5, kvT, 0.0).astype(BF16)
        wk2_s[:, d0:d1] = lax.dot_general(wob_s[e0:e1, :], kvT, TN,
                                          preferred_element_type=F32).astype(BF16)
    z16_s[...] = jnp.where(zm_s[...] > 0.5, xp_s[M:M + 1, :], 0.0).astype(BF16)
    c_copy.wait()

    def head(h, carry):
        j = h // 2
        slot = j % 2

        @pl.when(h % 2 == 0)
        def _():
            for cp in w_copies(j, slot):
                cp.wait()

            @pl.when(j + 1 < H // 2)
            def _():
                for cp in w_copies(j + 1, 1 - slot):
                    cp.start()

        shift = ((1 - h % 2) * 16).astype(U32)

        def unpack(buf):
            u = buf[slot]
            return lax.bitcast_convert_type((u << shift) & jnp.uint32(0xFFFF0000), F32)

        c = c_s[...]
        k_s[...] = _dot(c, unpack(wk_b).astype(BF16)).astype(BF16)
        wqT = unpack(wq_b).T.astype(BF16)
        qT_s[...] = (_dot(wqT, xT_s[...]) * (D ** -0.5)).astype(BF16)
        vT_s[...] = _dot(c, unpack(wv_b).astype(BF16)).T.astype(BF16)

        krow = lax.broadcasted_iota(jnp.int32, (TQ, TQ), 0)
        qcol = lax.broadcasted_iota(jnp.int32, (TQ, TQ), 1)
        causal = krow <= qcol

        def scores(i):
            lo = i * TQ
            s = _dot(k_s[0:lo + TQ, :], qT_s[:, lo:lo + TQ])
            s_d = jnp.where(causal, s[lo:lo + TQ], -1e9)
            m = jnp.max(s_d, axis=0, keepdims=True)
            s_o = None
            if i > 0:
                s_o = s[0:lo]
                m = jnp.maximum(m, jnp.max(s_o, axis=0, keepdims=True))
            return s_d, s_o, m

        def finish(i, s_d, s_o, m):
            lo = i * TQ
            p_d = jnp.exp(s_d - m)
            l = jnp.sum(p_d, axis=0, keepdims=True)
            p = p_d.astype(BF16)
            if i > 0:
                p_o = jnp.exp(s_o - m)
                l = l + jnp.sum(p_o, axis=0, keepdims=True)
                p = jnp.concatenate([p_o.astype(BF16), p], axis=0)
            ctxT = _dot(vT_s[:, 0:lo + TQ], p)
            ctxT_s[:, lo:lo + TQ] = (ctxT * (g_s[0:1, lo:lo + TQ] / l)).astype(BF16)

        pend = [scores(i) for i in range(NQ)]
        for i in range(NQ):
            finish(i, *pend[i])

        acc_s[...] += _dot(woT_b[slot, h % 2], ctxT_s[...])
        return carry

    lax.fori_loop(0, H, head, 0)

    def phase2(t, carry):
        off = pl.multiple_of(t * CB, CB)
        pq = pqT_s[:, pl.ds(off, CB)]
        den16 = _dot(z16_s[...], pq) + 1e-6
        rinv = 1.0 / den16
        r_hi = rinv.astype(BF16)
        r_lo = (rinv - r_hi.astype(F32)).astype(BF16)
        rfull = _dot(e2_s[...], jnp.concatenate([r_hi, r_lo], axis=0))
        oT = (pq.astype(F32) * rfull).astype(BF16)
        bT = _dot(wk2_s[...], oT)
        g = g_s[0:1, pl.ds(off, CB)]
        o_s[:, pl.ds(off, CB)] = (acc_s[:, pl.ds(off, CB)] + (1.0 - g) * bT).astype(BF16)
        o_copy(t).start()
        return carry

    lax.fori_loop(0, NCB, phase2, 0)
    for t in range(NCB):
        o_copy(t).wait()


@jax.jit
def pallas_gated_mix__compressed_kv_cla__linear_attn_block__prompt_kernel(
    A_x, A_c_kv, A_w_q, A_w_uk, A_w_uv, A_w_o, B_x, B_wqkv, B_wo, gate_w,
):
    xT = jnp.swapaxes(A_x, 1, 2)
    woT = jnp.swapaxes(A_w_o, 1, 2)
    ne = [e1 - e0 for (e0, e1) in _ER]
    nd = [d1 - d0 for (d0, d1) in _DT]
    any_spec = pl.BlockSpec(memory_space=pl.ANY)
    outT = pl.pallas_call(
        _kernel,
        in_specs=[any_spec] * 8 + [pl.BlockSpec(memory_space=pltpu.VMEM)],
        out_specs=any_spec,
        out_shape=jax.ShapeDtypeStruct((1, M, S), BF16),
        scratch_shapes=[
            pltpu.VMEM((M, S), BF16),
            pltpu.VMEM((S, DC), BF16),
            pltpu.VMEM((M, 3 * M), BF16),
            pltpu.VMEM((M, M), BF16),
            pltpu.VMEM((2, 2, M, D), BF16),
            pltpu.VMEM((2, M, D), U32),
            pltpu.VMEM((2, DC, D), U32),
            pltpu.VMEM((2, DC, D), U32),
            pltpu.SemaphoreType.DMA((NSEM,)),
            pltpu.VMEM((D, S), BF16),
            pltpu.VMEM((S, D), BF16),
            pltpu.VMEM((D, S), BF16),
            pltpu.VMEM((D, S), BF16),
            pltpu.VMEM((M, S), F32),
            pltpu.VMEM((3 * M + 16, M), BF16),
            pltpu.VMEM((M + 16, M), F32),
            pltpu.VMEM((M, S), BF16),
            pltpu.VMEM((16, M), BF16),
            pltpu.VMEM((16, M), F32),
            pltpu.VMEM((M, 32), BF16),
        ] + [pltpu.VMEM((ne[t], nd[t]), F32) for t in range(4)] + [
            pltpu.VMEM((M, M), BF16),
            pltpu.VMEM((8, S), F32),
            pltpu.VMEM((M, S), BF16),
        ],
        compiler_params=pltpu.CompilerParams(
            vmem_limit_bytes=100 * 1024 * 1024,
        ),
    )(xT, A_c_kv, A_w_q, A_w_uk, A_w_uv, woT, B_wqkv, B_wo, gate_w)
    return jnp.swapaxes(outT, 1, 2)
```

```python
import jax
import jax.numpy as jnp
from jax import lax
import jax.experimental.pallas as pl
import jax.experimental.pallas.tpu as pltpu

F32 = jnp.float32
BF16 = jnp.bfloat16
U32 = jnp.uint32

S = 2048
M = 448
H = 16
D = 256
DC = 1024
HB = 16
DH = M // HB
TQ = 128
NQ = S // TQ
CB = 512
NCB = S // CB

NT = (((1,), (1,)), ((), ()))
TN = (((0,), (0,)), ((), ()))

_DT = [(0, 128), (128, 256), (256, 384), (384, 448)]
_ER = []
for (_d0, _d1) in _DT:
    _h0, _h1 = _d0 // DH, (_d1 - 1) // DH
    _ER.append(((_h0 * DH) // 16 * 16, -(-((_h1 + 1) * DH) // 16) * 16))

SEM_W = 0
SEM_C = 8
SEM_WQKV = 9
SEM_WOB = 10
SEM_WQK = 11
SEM_X = 15
SEM_O = SEM_X + NCB
NSEM = SEM_O + NCB

GROW = 2 * M
VROW = 2 * M + 16


def _dot(a, b):
    return jnp.dot(a, b, preferred_element_type=F32)


def _hd(i):
    return (i * 2341) >> 16


assert all(((i * 2341) >> 16) == i // DH for i in range(512))


def _kernel(xT_hbm, c_hbm, wq_hbm, wk_hbm, wv_hbm, woT_hbm, wqkv_hbm, wob_hbm, gw_ref,
            out_hbm,
            xT_s, c_s, wqkv_s, wob_s, woT_b, wq_b, wk_b, wv_b, sems,
            qT_s, k_s, vT_s, ctxT_s, acc_s,
            wT_s, xp_s, pqT_s, zm_s, e2_s, mk0, mk1, mk2, mk3, wk2_s, g_s, o_s):
    mk = (mk0, mk1, mk2, mk3)

    def w_copies(jj, sl):
        return [
            pltpu.make_async_copy(wk_hbm.bitcast(U32).at[:, jj, :], wk_b.at[sl], sems.at[SEM_W + sl * 4 + 0]),
            pltpu.make_async_copy(wv_hbm.bitcast(U32).at[:, jj, :], wv_b.at[sl], sems.at[SEM_W + sl * 4 + 1]),
            pltpu.make_async_copy(wq_hbm.bitcast(U32).at[:, jj, :], wq_b.at[sl], sems.at[SEM_W + sl * 4 + 2]),
            pltpu.make_async_copy(woT_hbm.at[pl.ds(2 * jj, 2)], woT_b.at[sl], sems.at[SEM_W + sl * 4 + 3]),
        ]

    def x_copy(t):
        off = pl.multiple_of(t * CB, CB)
        return pltpu.make_async_copy(xT_hbm.at[0, :, pl.ds(off, CB)], xT_s.at[:, pl.ds(off, CB)],
                                     sems.at[SEM_X + t])

    def o_copy(t):
        off = pl.multiple_of(t * CB, CB)
        return pltpu.make_async_copy(o_s.at[:, pl.ds(off, CB)], out_hbm.at[0, :, pl.ds(off, CB)],
                                     sems.at[SEM_O + t])

    c_copy = pltpu.make_async_copy(c_hbm.at[0], c_s, sems.at[SEM_C])
    wv_copy = pltpu.make_async_copy(wqkv_hbm.at[:, 2 * M:3 * M], wqkv_s.at[:, 2 * M:3 * M], sems.at[SEM_WQKV])
    wqk_copies = [
        pltpu.make_async_copy(wqkv_hbm.at[112 * r:112 * (r + 1), 0:2 * M],
                              wqkv_s.at[112 * r:112 * (r + 1), 0:2 * M], sems.at[SEM_WQK + r])
        for r in range(4)]
    wob_copy = pltpu.make_async_copy(wob_hbm, wob_s, sems.at[SEM_WOB])
    for cp in wqk_copies:
        cp.start()
    x_copy(0).start()

    def phi(t):
        return jnp.where(t > 0, t + 1.0, jnp.exp(t)) + 1e-6

    xp_s[...] = jnp.zeros_like(xp_s)
    acc_s[...] = jnp.zeros_like(acc_s)
    for tt in range(4):
        (d0, d1), (e0, e1) = _DT[tt], _ER[tt]
        r = _hd(lax.broadcasted_iota(jnp.int32, (e1 - e0, d1 - d0), 0) + e0)
        cc = _hd(lax.broadcasted_iota(jnp.int32, (e1 - e0, d1 - d0), 1) + d0)
        mk[tt][...] = jnp.where(r == cc, 1.0, 0.0)
    hrow = lax.broadcasted_iota(jnp.int32, (16, M), 0)
    hcol = _hd(lax.broadcasted_iota(jnp.int32, (16, M), 1))
    zm_s[...] = jnp.where(hrow == hcol, 1.0, 0.0)
    erow = _hd(lax.broadcasted_iota(jnp.int32, (M, 32), 0))
    ecol = lax.broadcasted_iota(jnp.int32, (M, 32), 1) & 15
    e2_s[...] = jnp.where(erow == ecol, 1.0, 0.0).astype(BF16)
    wT_s[GROW:GROW + 16, :] = jnp.broadcast_to(gw_ref[...].reshape(1, M), (16, M))

    for cp in wqk_copies:
        cp.wait()
    wv_copy.start()
    wob_copy.start()
    for t in range(1, NCB):
        x_copy(t).start()
    c_copy.start()
    for cp in w_copies(0, 0):
        cp.start()
    wT_s[0:2 * M, :] = wqkv_s[:, 0:2 * M].astype(F32).T.astype(BF16)

    def phase1(t, carry):
        off = pl.multiple_of(t * CB, CB)
        x_copy(t).wait()
        xT = xT_s[:, pl.ds(off, CB)]
        qkT = _dot(wT_s[0:VROW, :], xT)
        qbT = qkT[0:M].astype(BF16).astype(F32)
        kbT = qkT[M:2 * M].astype(BF16).astype(F32)
        g_s[:, pl.ds(off, CB)] = jax.nn.sigmoid(qkT[GROW:GROW + 8])
        pqT_s[:, pl.ds(off, CB)] = phi(qbT).astype(BF16)
        pkT = phi(kbT).astype(BF16)
        xaug = jnp.concatenate([xT, jnp.ones((16, CB), BF16)], axis=0)
        xp_s[...] += lax.dot_general(xaug, pkT, NT, preferred_element_type=F32)
        return carry

    lax.fori_loop(0, NCB, phase1, 0)

    wob_copy.wait()
    wv_copy.wait()
    wT_s[VROW:VROW + M, :] = wqkv_s[:, 2 * M:3 * M].astype(F32).T.astype(BF16)
    for tt in range(4):
        (d0, d1), (e0, e1) = _DT[tt], _ER[tt]
        kvT = _dot(wT_s[VROW + e0:VROW + e1, :], xp_s[0:M, d0:d1].astype(BF16))
        kvT = jnp.where(mk[tt][...] > 0.5, kvT, 0.0).astype(BF16)
        wk2_s[:, d0:d1] = lax.dot_general(wob_s[e0:e1, :], kvT, TN,
                                          preferred_element_type=F32).astype(BF16)
    z16 = jnp.where(zm_s[...] > 0.5, xp_s[M:M + 1, :], 0.0).astype(BF16)
    pq = pqT_s[...]
    den16 = _dot(z16, pq) + 1e-6
    rinv = 1.0 / den16
    r_hi = rinv.astype(BF16)
    r_lo = (rinv - r_hi.astype(F32)).astype(BF16)
    rfull = _dot(e2_s[...], jnp.concatenate([r_hi, r_lo], axis=0))
    pqT_s[...] = (pq.astype(F32) * rfull).astype(BF16)
    c_copy.wait()

    def head(h, carry):
        j = h // 2
        slot = j % 2

        @pl.when(h % 2 == 0)
        def _():
            for cp in w_copies(j, slot):
                cp.wait()

            @pl.when(j + 1 < H // 2)
            def _():
                for cp in w_copies(j + 1, 1 - slot):
                    cp.start()

        shift = ((1 - h % 2) * 16).astype(U32)

        def unpack(buf):
            u = buf[slot]
            return lax.bitcast_convert_type((u << shift) & jnp.uint32(0xFFFF0000), F32)

        c = c_s[...]
        k_s[...] = _dot(c, unpack(wk_b).astype(BF16)).astype(BF16)
        wqT = unpack(wq_b).T.astype(BF16)
        qT_s[...] = (_dot(wqT, xT_s[...]) * (D ** -0.5)).astype(BF16)

        krow = lax.broadcasted_iota(jnp.int32, (TQ, TQ), 0)
        qcol = lax.broadcasted_iota(jnp.int32, (TQ, TQ), 1)
        causal = krow <= qcol

        def scores(i):
            lo = i * TQ
            s = _dot(k_s[0:lo + TQ, :], qT_s[:, lo:lo + TQ])
            s_d = jnp.where(causal, s[lo:lo + TQ], -1e9)
            m = jnp.max(s_d, axis=0, keepdims=True)
            s_o = None
            if i > 0:
                s_o = s[0:lo]
                m = jnp.maximum(m, jnp.max(s_o, axis=0, keepdims=True))
            return s_d, s_o, m

        def finish(i, s_d, s_o, m):
            lo = i * TQ
            p_d = jnp.exp(s_d - m)
            l = jnp.sum(p_d, axis=0, keepdims=True)
            p = p_d.astype(BF16)
            if i > 0:
                p_o = jnp.exp(s_o - m)
                l = l + jnp.sum(p_o, axis=0, keepdims=True)
                p = jnp.concatenate([p_o.astype(BF16), p], axis=0)
            ctxT = _dot(vT_s[:, 0:lo + TQ], p)
            ctxT_s[:, lo:lo + TQ] = (ctxT * (g_s[0:1, lo:lo + TQ] / l)).astype(BF16)

        pend = [scores(i) for i in range(NQ)]
        vT_s[...] = _dot(c, unpack(wv_b).astype(BF16)).T.astype(BF16)
        for i in range(NQ):
            finish(i, *pend[i])

        acc_s[...] += _dot(woT_b[slot, h % 2], ctxT_s[...])
        return carry

    lax.fori_loop(0, H, head, 0)

    def phase2(t, carry):
        off = pl.multiple_of(t * CB, CB)
        bT = _dot(wk2_s[...], pqT_s[:, pl.ds(off, CB)])
        g = g_s[0:1, pl.ds(off, CB)]
        o_s[:, pl.ds(off, CB)] = (acc_s[:, pl.ds(off, CB)] + (1.0 - g) * bT).astype(BF16)
        o_copy(t).start()
        return carry

    lax.fori_loop(0, NCB, phase2, 0)
    for t in range(NCB):
        o_copy(t).wait()


@jax.jit
def pallas_gated_mix__compressed_kv_cla__linear_attn_block__prompt_kernel(
    A_x, A_c_kv, A_w_q, A_w_uk, A_w_uv, A_w_o, B_x, B_wqkv, B_wo, gate_w,
):
    xT = jnp.swapaxes(A_x, 1, 2)
    woT = jnp.swapaxes(A_w_o, 1, 2)
    ne = [e1 - e0 for (e0, e1) in _ER]
    nd = [d1 - d0 for (d0, d1) in _DT]
    any_spec = pl.BlockSpec(memory_space=pl.ANY)
    outT = pl.pallas_call(
        _kernel,
        in_specs=[any_spec] * 8 + [pl.BlockSpec(memory_space=pltpu.VMEM)],
        out_specs=any_spec,
        out_shape=jax.ShapeDtypeStruct((1, M, S), BF16),
        scratch_shapes=[
            pltpu.VMEM((M, S), BF16),
            pltpu.VMEM((S, DC), BF16),
            pltpu.VMEM((M, 3 * M), BF16),
            pltpu.VMEM((M, M), BF16),
            pltpu.VMEM((2, 2, M, D), BF16),
            pltpu.VMEM((2, M, D), U32),
            pltpu.VMEM((2, DC, D), U32),
            pltpu.VMEM((2, DC, D), U32),
            pltpu.SemaphoreType.DMA((NSEM,)),
            pltpu.VMEM((D, S), BF16),
            pltpu.VMEM((S, D), BF16),
            pltpu.VMEM((D, S), BF16),
            pltpu.VMEM((D, S), BF16),
            pltpu.VMEM((M, S), F32),
            pltpu.VMEM((3 * M + 16, M), BF16),
            pltpu.VMEM((M + 16, M), F32),
            pltpu.VMEM((M, S), BF16),
            pltpu.VMEM((16, M), F32),
            pltpu.VMEM((M, 32), BF16),
        ] + [pltpu.VMEM((ne[t], nd[t]), F32) for t in range(4)] + [
            pltpu.VMEM((M, M), BF16),
            pltpu.VMEM((8, S), F32),
            pltpu.VMEM((M, S), BF16),
        ],
        compiler_params=pltpu.CompilerParams(
            vmem_limit_bytes=100 * 1024 * 1024,
        ),
    )(xT, A_c_kv, A_w_q, A_w_uk, A_w_uv, woT, B_wqkv, B_wo, gate_w)
    return jnp.swapaxes(outT, 1, 2)
```

```python
import jax
import jax.numpy as jnp
from jax import lax
import jax.experimental.pallas as pl
import jax.experimental.pallas.tpu as pltpu

F32 = jnp.float32
BF16 = jnp.bfloat16
U32 = jnp.uint32

S = 2048
M = 448
H = 16
D = 256
DC = 1024
HB = 16
DH = M // HB
TQ = 128
NQ = S // TQ
CB = 512
NCB = S // CB

NT = (((1,), (1,)), ((), ()))
TN = (((0,), (0,)), ((), ()))

_DT = [(0, 128), (128, 256), (256, 384), (384, 448)]
_ER = []
for (_d0, _d1) in _DT:
    _h0, _h1 = _d0 // DH, (_d1 - 1) // DH
    _ER.append(((_h0 * DH) // 16 * 16, -(-((_h1 + 1) * DH) // 16) * 16))

SEM_W = 0
SEM_C = 8
SEM_WQKV = 9
SEM_WOB = 10
SEM_WQK = 11
SEM_X = 15
SEM_O = SEM_X + NCB
NSEM = SEM_O + NCB

GROW = 2 * M
VROW = 2 * M + 16


def _dot(a, b):
    return jnp.dot(a, b, preferred_element_type=F32)


def _hd(i):
    return (i * 2341) >> 16


assert all(((i * 2341) >> 16) == i // DH for i in range(512))


def _kernel(xT_hbm, c_hbm, wq_hbm, wk_hbm, wv_hbm, woT_hbm, wqkv_hbm, wob_hbm, gw_ref,
            out_hbm,
            xT_s, c_s, wqkv_s, wob_s, woT_b, wq_b, wk_b, wv_b, sems,
            qT_s, k_s, vT_s, ctxT_s, acc_s,
            wT_s, xp_s, pqT_s, zm_s, mk0, mk1, mk2, mk3, wk2_s, g_s, o_s):
    mk = (mk0, mk1, mk2, mk3)

    def w_copies(jj, sl):
        return [
            pltpu.make_async_copy(wk_hbm.bitcast(U32).at[:, jj, :], wk_b.at[sl], sems.at[SEM_W + sl * 4 + 0]),
            pltpu.make_async_copy(wv_hbm.bitcast(U32).at[:, jj, :], wv_b.at[sl], sems.at[SEM_W + sl * 4 + 1]),
            pltpu.make_async_copy(wq_hbm.bitcast(U32).at[:, jj, :], wq_b.at[sl], sems.at[SEM_W + sl * 4 + 2]),
            pltpu.make_async_copy(woT_hbm.at[pl.ds(2 * jj, 2)], woT_b.at[sl], sems.at[SEM_W + sl * 4 + 3]),
        ]

    def x_copy(t):
        off = pl.multiple_of(t * CB, CB)
        return pltpu.make_async_copy(xT_hbm.at[0, :, pl.ds(off, CB)], xT_s.at[:, pl.ds(off, CB)],
                                     sems.at[SEM_X + t])

    def o_copy(t):
        off = pl.multiple_of(t * CB, CB)
        return pltpu.make_async_copy(o_s.at[:, pl.ds(off, CB)], out_hbm.at[0, :, pl.ds(off, CB)],
                                     sems.at[SEM_O + t])

    c_copy = pltpu.make_async_copy(c_hbm.at[0], c_s, sems.at[SEM_C])
    wv_copy = pltpu.make_async_copy(wqkv_hbm.at[:, 2 * M:3 * M], wqkv_s.at[:, 2 * M:3 * M], sems.at[SEM_WQKV])
    wqk_copies = [
        pltpu.make_async_copy(wqkv_hbm.at[112 * r:112 * (r + 1), 0:2 * M],
                              wqkv_s.at[112 * r:112 * (r + 1), 0:2 * M], sems.at[SEM_WQK + r])
        for r in range(4)]
    wob_copy = pltpu.make_async_copy(wob_hbm, wob_s, sems.at[SEM_WOB])
    for cp in wqk_copies:
        cp.start()
    x_copy(0).start()

    def phi(t):
        return jnp.where(t > 0, t + 1.0, jnp.exp(t)) + 1e-6

    xp_s[...] = jnp.zeros_like(xp_s)
    acc_s[...] = jnp.zeros_like(acc_s)
    for tt in range(4):
        (d0, d1), (e0, e1) = _DT[tt], _ER[tt]
        r = _hd(lax.broadcasted_iota(jnp.int32, (e1 - e0, d1 - d0), 0) + e0)
        cc = _hd(lax.broadcasted_iota(jnp.int32, (e1 - e0, d1 - d0), 1) + d0)
        mk[tt][...] = jnp.where(r == cc, 1.0, 0.0)
    hrow = lax.broadcasted_iota(jnp.int32, (16, M), 0)
    hcol = _hd(lax.broadcasted_iota(jnp.int32, (16, M), 1))
    zm_s[...] = jnp.where(hrow == hcol, 1.0, 0.0)
    wT_s[GROW:GROW + 16, :] = jnp.broadcast_to(gw_ref[...].reshape(1, M), (16, M))

    for cp in wqk_copies:
        cp.wait()
    wv_copy.start()
    wob_copy.start()
    for t in range(1, NCB):
        x_copy(t).start()
    c_copy.start()
    for cp in w_copies(0, 0):
        cp.start()
    wT_s[0:2 * M, :] = wqkv_s[:, 0:2 * M].astype(F32).T.astype(BF16)

    def phase1(t, carry):
        off = pl.multiple_of(t * CB, CB)
        x_copy(t).wait()
        xT = xT_s[:, pl.ds(off, CB)]
        qkT = _dot(wT_s[0:VROW, :], xT)
        qbT = qkT[0:M].astype(BF16).astype(F32)
        kbT = qkT[M:2 * M].astype(BF16).astype(F32)
        g_s[:, pl.ds(off, CB)] = jax.nn.sigmoid(qkT[GROW:GROW + 8])
        pqT_s[:, pl.ds(off, CB)] = phi(qbT).astype(BF16)
        pkT = phi(kbT).astype(BF16)
        xaug = jnp.concatenate([xT, jnp.ones((16, CB), BF16)], axis=0)
        xp_s[...] += lax.dot_general(xaug, pkT, NT, preferred_element_type=F32)
        return carry

    lax.fori_loop(0, NCB, phase1, 0)

    wob_copy.wait()
    wv_copy.wait()
    wT_s[VROW:VROW + M, :] = wqkv_s[:, 2 * M:3 * M].astype(F32).T.astype(BF16)
    for tt in range(4):
        (d0, d1), (e0, e1) = _DT[tt], _ER[tt]
        kvT = _dot(wT_s[VROW + e0:VROW + e1, :], xp_s[0:M, d0:d1].astype(BF16))
        kvT = jnp.where(mk[tt][...] > 0.5, kvT, 0.0).astype(BF16)
        wk2_s[:, d0:d1] = lax.dot_general(wob_s[e0:e1, :], kvT, TN,
                                          preferred_element_type=F32).astype(BF16)
    z16 = jnp.where(zm_s[...] > 0.5, xp_s[M:M + 1, :], 0.0).astype(BF16)
    pq = pqT_s[...]
    den16 = _dot(z16, pq) + 1e-6
    rinv = 1.0 / den16
    rfull = jnp.concatenate([jnp.broadcast_to(rinv[hh:hh + 1, :], (DH, S)) for hh in range(HB)], axis=0)
    pqT_s[...] = (pq.astype(F32) * rfull).astype(BF16)
    c_copy.wait()

    def head(h, carry):
        j = h // 2
        slot = j % 2

        @pl.when(h % 2 == 0)
        def _():
            for cp in w_copies(j, slot):
                cp.wait()

            @pl.when(j + 1 < H // 2)
            def _():
                for cp in w_copies(j + 1, 1 - slot):
                    cp.start()

        shift = ((1 - h % 2) * 16).astype(U32)

        def unpack(buf):
            u = buf[slot]
            return lax.bitcast_convert_type((u << shift) & jnp.uint32(0xFFFF0000), F32)

        c = c_s[...]
        k_s[...] = _dot(c, unpack(wk_b).astype(BF16)).astype(BF16)
        wqT = unpack(wq_b).T.astype(BF16)
        qT_s[...] = (_dot(wqT, xT_s[...]) * (D ** -0.5)).astype(BF16)

        krow = lax.broadcasted_iota(jnp.int32, (TQ, TQ), 0)
        qcol = lax.broadcasted_iota(jnp.int32, (TQ, TQ), 1)
        causal = krow <= qcol

        def scores(i):
            lo = i * TQ
            s = _dot(k_s[0:lo + TQ, :], qT_s[:, lo:lo + TQ])
            s_d = jnp.where(causal, s[lo:lo + TQ], -1e9)
            m = jnp.max(s_d, axis=0, keepdims=True)
            s_o = None
            if i > 0:
                s_o = s[0:lo]
                m = jnp.maximum(m, jnp.max(s_o, axis=0, keepdims=True))
            return s_d, s_o, m

        def finish(i, s_d, s_o, m):
            lo = i * TQ
            p_d = jnp.exp(s_d - m)
            l = jnp.sum(p_d, axis=0, keepdims=True)
            p = p_d.astype(BF16)
            if i > 0:
                p_o = jnp.exp(s_o - m)
                l = l + jnp.sum(p_o, axis=0, keepdims=True)
                p = jnp.concatenate([p_o.astype(BF16), p], axis=0)
            ctxT = _dot(vT_s[:, 0:lo + TQ], p)
            ctxT_s[:, lo:lo + TQ] = (ctxT * (g_s[0:1, lo:lo + TQ] / l)).astype(BF16)

        pend = [scores(i) for i in range(NQ)]
        vT_s[...] = _dot(c, unpack(wv_b).astype(BF16)).T.astype(BF16)
        for i in range(NQ):
            finish(i, *pend[i])

        acc_s[...] += _dot(woT_b[slot, h % 2], ctxT_s[...])
        return carry

    lax.fori_loop(0, H, head, 0)

    def phase2(t, carry):
        off = pl.multiple_of(t * CB, CB)
        bT = _dot(wk2_s[...], pqT_s[:, pl.ds(off, CB)])
        g = g_s[0:1, pl.ds(off, CB)]
        o_s[:, pl.ds(off, CB)] = (acc_s[:, pl.ds(off, CB)] + (1.0 - g) * bT).astype(BF16)
        o_copy(t).start()
        return carry

    lax.fori_loop(0, NCB, phase2, 0)
    for t in range(NCB):
        o_copy(t).wait()


@jax.jit
def pallas_gated_mix__compressed_kv_cla__linear_attn_block__prompt_kernel(
    A_x, A_c_kv, A_w_q, A_w_uk, A_w_uv, A_w_o, B_x, B_wqkv, B_wo, gate_w,
):
    xT = jnp.swapaxes(A_x, 1, 2)
    woT = jnp.swapaxes(A_w_o, 1, 2)
    ne = [e1 - e0 for (e0, e1) in _ER]
    nd = [d1 - d0 for (d0, d1) in _DT]
    any_spec = pl.BlockSpec(memory_space=pl.ANY)
    outT = pl.pallas_call(
        _kernel,
        in_specs=[any_spec] * 8 + [pl.BlockSpec(memory_space=pltpu.VMEM)],
        out_specs=any_spec,
        out_shape=jax.ShapeDtypeStruct((1, M, S), BF16),
        scratch_shapes=[
            pltpu.VMEM((M, S), BF16),
            pltpu.VMEM((S, DC), BF16),
            pltpu.VMEM((M, 3 * M), BF16),
            pltpu.VMEM((M, M), BF16),
            pltpu.VMEM((2, 2, M, D), BF16),
            pltpu.VMEM((2, M, D), U32),
            pltpu.VMEM((2, DC, D), U32),
            pltpu.VMEM((2, DC, D), U32),
            pltpu.SemaphoreType.DMA((NSEM,)),
            pltpu.VMEM((D, S), BF16),
            pltpu.VMEM((S, D), BF16),
            pltpu.VMEM((D, S), BF16),
            pltpu.VMEM((D, S), BF16),
            pltpu.VMEM((M, S), F32),
            pltpu.VMEM((3 * M + 16, M), BF16),
            pltpu.VMEM((M + 16, M), F32),
            pltpu.VMEM((M, S), BF16),
            pltpu.VMEM((16, M), F32),
        ] + [pltpu.VMEM((ne[t], nd[t]), F32) for t in range(4)] + [
            pltpu.VMEM((M, M), BF16),
            pltpu.VMEM((8, S), F32),
            pltpu.VMEM((M, S), BF16),
        ],
        compiler_params=pltpu.CompilerParams(
            vmem_limit_bytes=100 * 1024 * 1024,
        ),
    )(xT, A_c_kv, A_w_q, A_w_uk, A_w_uv, woT, B_wqkv, B_wo, gate_w)
    return jnp.swapaxes(outT, 1, 2)
```
